```python
import os as _os
_os.environ.setdefault("JAX_PLATFORMS", "cpu")
import jax
import jax.numpy as jnp

def _softmax(x, axis=-1):
    return jax.nn.softmax(x, axis=axis)
def _gelu(x):
    return jax.nn.gelu(x, approximate=True)
def _silu(x):
    return jax.nn.silu(x)
def _sigmoid(x):
    return jax.nn.sigmoid(x)
def _layernorm(x, axis=-1, eps=1e-5):
    m = jnp.mean(x, axis=axis, keepdims=True)
    v = jnp.var(x, axis=axis, keepdims=True)
    return (x - m) / jnp.sqrt(v + eps)
def _scatter_add(tgt, idx, src, axis=0):
    return tgt.at[idx].add(src)
def _segment_sum(src, seg, n):
    return jax.ops.segment_sum(src, seg, n)
class _Rng:
    def __init__(self, key):
        self._k = key
    def _next(self):
        self._k, sub = jax.random.split(self._k)
        return sub
    def normal(self, shape):
        return jax.random.normal(self._next(), shape, dtype=jnp.bfloat16)
    def randint(self, lo, hi, shape):
        return jax.random.randint(self._next(), shape, lo, hi, dtype=jnp.int32)
    def uniform(self, shape, lo=0.0, hi=1.0):
        return jax.random.uniform(self._next(), shape, jnp.bfloat16, lo, hi)
    def permutation(self, n):
        return jax.random.permutation(self._next(), n)


kernel_name = 'gated_mix__sliding_block_cached__swiglu_ffn__decode'

def setup_inputs():
    _rng = _Rng(jax.random.key(int.from_bytes(__import__("os").urandom(4), "little")))
    _w = (lambda a: (lambda t: t.astype(jnp.bfloat16) if jnp.issubdtype(t.dtype, jnp.floating) else t)(jnp.asarray(a)))
    def _A_setup():
        B, Sq, D = 1, 1, 512
        Hq, Hkv, Sk, Dh = 32, 32, 32768, 128
        assert Hq % Hkv == 0, (Hq, Hkv)
        return {
            "x": _w((lambda *s: _rng.normal(s) * 0.05)(B, Sq, D)),
            "k_cache": _w((lambda *s: _rng.normal(s) * 3.2)(B, Hkv, Sk, Dh)),
            "v_cache": _w((lambda *s: _rng.normal(s) * 1.6)(B, Hkv, Sk, Dh)),
            "wq": _w((lambda *s: _rng.normal(s) * 3.2)(D, Hq * Dh) * (D ** -0.5)),
            "wo": _w((lambda *s: _rng.normal(s) * 1.6)(Hq * Dh, D) * ((Hq * Dh) ** -0.5)),
        }
    _A_in = _A_setup()

    def _B_setup():
        B, S, D, F = 1, 1, 512, 1376
        return {
            "x": _w((lambda *s: _rng.normal(s) * 0.05)(B, S, D)),
            "w_gate": _w((lambda *s: _rng.normal(s) * 0.1)(D, F)),
            "w_up": _w((lambda *s: _rng.normal(s) * 0.1)(D, F)),
            "w_down": _w((lambda *s: _rng.normal(s) * 0.1)(F, D)),
        }
    _B_in = _B_setup()

    return {
        "A_x": _A_in["x"],
        "A_k_cache": _A_in["k_cache"],
        "A_v_cache": _A_in["v_cache"],
        "A_wq": _A_in["wq"],
        "A_wo": _A_in["wo"],
        "B_x": _B_in["x"],
        "B_w_gate": _B_in["w_gate"],
        "B_w_up": _B_in["w_up"],
        "B_w_down": _B_in["w_down"],
        "gate_w": _w((lambda *s: _rng.normal(s) * 0.05)(512) * 16.0),
    }

def reference(A_x, A_k_cache, A_v_cache, A_wq, A_wo, B_x, B_w_gate, B_w_up, B_w_down, gate_w):
    def _A_ref(x, k_cache, v_cache, wq, wo):
        B, Sq, D = x.shape
        Hq, Dh = 32, 128
        Hkv, Sk = k_cache.shape[1], k_cache.shape[2]
        W = min(4096, max(256, Sk // 4))
        rep = Hq // Hkv
        q = (lambda x, *d: x.transpose(*d))((x @ wq).reshape(B, Sq, Hq, Dh), 0, 2, 1, 3)
        k = jnp.repeat(k_cache[:, :, Sk - W:, :], rep, axis=1)
        v = jnp.repeat(v_cache[:, :, Sk - W:, :], rep, axis=1)
        scores = jnp.einsum("bhqd,bhkd->bhqk", q, k) * (Dh ** -0.5)
        p = _softmax(scores, axis=-1)
        o = jnp.einsum("bhqk,bhkd->bhqd", p, v)
        return (lambda x, *d: x.transpose(*d))(o, 0, 2, 1, 3).reshape(B, Sq, Hq * Dh) @ wo

    def _B_ref(x, w_gate, w_up, w_down):
        g = _silu(x @ w_gate)
        u = x @ w_up
        return (g * u) @ w_down

    x = A_x
    g = _sigmoid((x * gate_w).sum(-1, keepdims=True))
    a = _A_ref(x, A_k_cache, A_v_cache, A_wq, A_wo)
    b = _B_ref(x, B_w_gate, B_w_up, B_w_down)
    return g * a + (1 - g) * b
```

```python
import jax
import jax.numpy as jnp
from jax import lax
import jax.experimental.pallas as pl
import jax.experimental.pallas.tpu as pltpu

_NT = (((1,), (1,)), ((), ()))
_M = 8
_KV_GROUPS = (8, 8, 8, 8)
_WO_PIECES = (16, 8, 4, 2, 2)


@jax.jit
def pallas_gated_mix__sliding_block_cached__swiglu_ffn__decode_kernel(
    A_x: jax.Array,
    A_k_cache: jax.Array,
    A_v_cache: jax.Array,
    A_wq: jax.Array,
    A_wo: jax.Array,
    B_x: jax.Array,
    B_w_gate: jax.Array,
    B_w_up: jax.Array,
    B_w_down: jax.Array,
    gate_w: jax.Array,
):
    del B_x
    f32, bf16 = jnp.float32, jnp.bfloat16
    _, _, D = A_x.shape
    _, H, SK, DH = A_k_cache.shape
    F = B_w_down.shape[0]
    W = min(4096, max(256, SK // 4))
    scale = DH ** -0.5
    assert sum(_KV_GROUPS) == H and sum(_WO_PIECES) == H

    def kernel(x_hbm, k_hbm, v_hbm, wq_hbm, wo_hbm, wg_hbm, wu_hbm, wd_hbm, gw_hbm, out_ref,
               xb, gwb, kb, vb, wqb, wob, wgb, wub, wdb, q_scr, p_scr, l_scr, o_scr, sems):
        started = []

        def fetch(src, dst):
            copy = pltpu.make_async_copy(src, dst, sems.at[len(started)])
            copy.start()
            started.append(copy)
            return copy

        c_wq = fetch(wq_hbm, wqb)
        c_x = fetch(x_hbm, xb)
        c_gw = fetch(gw_hbm, gwb)
        c_k, c_v = [], []
        h0 = 0
        for g in _KV_GROUPS:
            c_k.append(fetch(k_hbm.at[0, pl.ds(h0, g), pl.ds(SK - W, W), :], kb.at[pl.ds(h0, g)]))
            c_v.append(fetch(v_hbm.at[0, pl.ds(h0, g), pl.ds(SK - W, W), :], vb.at[pl.ds(h0, g)]))
            h0 += g
        c_wg = fetch(wg_hbm, wgb)
        c_wu = fetch(wu_hbm, wub)
        c_wd = fetch(wd_hbm, wdb)
        c_wo = []
        h0 = 0
        for g in _WO_PIECES:
            c_wo.append(fetch(wo_hbm.at[pl.ds(h0 * DH, g * DH)], wob.at[pl.ds(h0 * DH, g * DH)]))
            h0 += g

        c_x.wait()
        c_gw.wait()
        x1 = xb[0].astype(f32)
        gw1 = gwb[...].astype(f32).reshape(1, D)
        gate = jax.nn.sigmoid(jnp.sum(x1 * gw1, axis=-1, keepdims=True))
        xm = jnp.broadcast_to(x1, (_M, D)).astype(bf16)

        def q_body(h, _):
            w = wqb[:, pl.ds(pl.multiple_of(h * DH, DH), DH)]
            q_scr[h] = jnp.dot(xm, w, preferred_element_type=f32)

        def qk_body(h, _):
            q = q_scr[h].astype(bf16)
            s = lax.dot_general(q, kb[h], _NT, preferred_element_type=f32) * scale
            p = jnp.exp(s - jnp.max(s, axis=-1, keepdims=True))
            p_scr[h] = p
            l_scr[h] = jnp.broadcast_to(jnp.sum(p, axis=-1, keepdims=True), (_M, DH))

        def pv_body(h, _):
            o = jnp.dot(p_scr[h].astype(bf16), vb[h], preferred_element_type=f32)
            o_scr[h] = o / l_scr[h]

        def wo_body(h, acc):
            w = wob[pl.ds(pl.multiple_of(h * DH, DH), DH), :]
            return acc + jnp.dot(o_scr[h].astype(bf16), w, preferred_element_type=f32)

        c_wq.wait()
        lax.fori_loop(0, H, q_body, None, unroll=4)
        h0 = 0
        for i, g in enumerate(_KV_GROUPS):
            c_k[i].wait()
            lax.fori_loop(h0, h0 + g, qk_body, None)
            c_v[i].wait()
            lax.fori_loop(h0, h0 + g, pv_body, None)
            h0 += g

        c_wg.wait()
        gg = lax.dot_general(xm, wgb[...], _NT, preferred_element_type=f32)
        c_wu.wait()
        uu = lax.dot_general(xm, wub[...], _NT, preferred_element_type=f32)
        hh = (gg * jax.nn.sigmoid(gg) * uu).astype(bf16)
        c_wd.wait()
        b = jnp.dot(hh, wdb[...], preferred_element_type=f32)

        acc = jnp.zeros((_M, D), f32)
        h0 = 0
        for i, g in enumerate(_WO_PIECES):
            c_wo[i].wait()
            if g > 2:
                acc = lax.fori_loop(h0, h0 + g, wo_body, acc, unroll=2)
            else:
                for h in range(h0, h0 + g):
                    acc = acc + jnp.dot(o_scr[h].astype(bf16), wob[h * DH:(h + 1) * DH, :],
                                        preferred_element_type=f32)
            h0 += g
        out_ref[0] = (gate * acc[0:1] + (1.0 - gate) * b[0:1]).astype(out_ref.dtype)

    hbm = pl.BlockSpec(memory_space=pltpu.HBM)
    return pl.pallas_call(
        kernel,
        out_shape=jax.ShapeDtypeStruct(A_x.shape, A_x.dtype),
        in_specs=[hbm] * 9,
        out_specs=pl.BlockSpec(memory_space=pltpu.VMEM),
        scratch_shapes=[
            pltpu.VMEM(A_x.shape, bf16), pltpu.VMEM(gate_w.shape, bf16),
            pltpu.VMEM((H, W, DH), bf16), pltpu.VMEM((H, W, DH), bf16),
            pltpu.VMEM(A_wq.shape, bf16), pltpu.VMEM(A_wo.shape, bf16),
            pltpu.VMEM((F, D), bf16), pltpu.VMEM((F, D), bf16), pltpu.VMEM((F, D), bf16),
            pltpu.VMEM((H, _M, DH), f32), pltpu.VMEM((H, _M, W), f32),
            pltpu.VMEM((H, _M, DH), f32), pltpu.VMEM((H, _M, DH), f32),
            pltpu.SemaphoreType.DMA((6 + 2 * len(_KV_GROUPS) + len(_WO_PIECES),)),
        ],
        compiler_params=pltpu.CompilerParams(vmem_limit_bytes=100 * 1024 * 1024),
    )(A_x, A_k_cache, A_v_cache, A_wq, A_wo, B_w_gate.T, B_w_up.T, B_w_down, gate_w)
```

```python
import jax
import jax.numpy as jnp
from jax import lax
import jax.experimental.pallas as pl
import jax.experimental.pallas.tpu as pltpu

_NT = (((1,), (1,)), ((), ()))
_M = 8
_G = 4
_ROWS = 32
_LEAD = 96
_LATE_STEP = 24
_WO_MXU = (16, 8, 4, 2, 1)
_WO_VPU = (96, 32)


def _round_robin(items, ways):
    run = -(-len(items) // ways)
    return [items[j] for i in range(run) for j in range(i, len(items), run)]


@jax.jit
def pallas_gated_mix__sliding_block_cached__swiglu_ffn__decode_kernel(
    A_x: jax.Array,
    A_k_cache: jax.Array,
    A_v_cache: jax.Array,
    A_wq: jax.Array,
    A_wo: jax.Array,
    B_x: jax.Array,
    B_w_gate: jax.Array,
    B_w_up: jax.Array,
    B_w_down: jax.Array,
    gate_w: jax.Array,
):
    del B_x
    f32, bf16 = jnp.float32, jnp.bfloat16
    _, _, D = A_x.shape
    _, H, SK, DH = A_k_cache.shape
    F = B_w_down.shape[0]
    W = min(4096, max(256, SK // 4))
    scale = DH ** -0.5
    n_groups = H // _G
    steps = W // _ROWS
    lead_steps = _LEAD // 2
    head_steps = (steps - lead_steps) // _G
    assert lead_steps + _G * head_steps == steps and n_groups * _G == H
    assert sum(_WO_MXU) == H - 1 and sum(_WO_VPU) == DH and F % _ROWS == 0
    wo_sizes = [n * DH for n in _WO_MXU] + list(_WO_VPU)
    wo_starts = [sum(wo_sizes[:i]) for i in range(len(wo_sizes))]
    s_wq, s_x, s_gw, s_wg, s_wu, s_wd, s_wo = range(2 * n_groups, 2 * n_groups + 7)

    def kernel(x_hbm, k_hbm, v_hbm, wq_hbm, wo_hbm, wg_hbm, wu_hbm, wd_hbm, gw_hbm, out_ref,
               xb, gwb, kb, vb, wqb, wob, wgb, wub, wdb, o_scr, ot_scr):
        def body(sems):
            def start(copies):
                for i, (src, dst, idx, s) in enumerate(copies):
                    pltpu.make_async_copy(src.at[idx], dst.at[idx], sems.at[s]).start(priority=i % 2)

            def wait_all(buf, s):
                pltpu.make_async_copy(buf, buf, sems.at[s]).wait()

            def row_copies(src, dst, first, n, s):
                return [(src, dst, (pl.ds(r, _ROWS),), s) for r in range(first, first + n, _ROWS)]

            def start_kv(g, first, n):
                heads = pl.ds(g * _G, _G)

                def step(i, _):
                    r = pl.multiple_of(i * _ROWS, _ROWS)
                    for j, (src, dst) in enumerate(((k_hbm, kb), (v_hbm, vb))):
                        pltpu.make_async_copy(
                            src.at[0, heads, pl.ds(SK - W + r, _ROWS), :],
                            dst.at[heads, pl.ds(r, _ROWS), :],
                            sems.at[2 * g + j],
                        ).start(priority=j)

                lax.fori_loop(first, first + n, step, None)

            def wait_kv(g):
                wait_all(kb.at[pl.ds(g * _G, _G)], 2 * g)
                wait_all(vb.at[pl.ds(g * _G, _G)], 2 * g + 1)

            early = _round_robin(
                [(wq_hbm, wqb, (pl.ds(r, _ROWS), pl.ds(c, D)), s_wq)
                 for r in range(0, D, _ROWS) for c in range(0, H * DH, D)], 8)
            late = _round_robin(
                row_copies(wg_hbm, wgb, 0, F, s_wg) + row_copies(wu_hbm, wub, 0, F, s_wu)
                + row_copies(wd_hbm, wdb, 0, F, s_wd), 6)
            for i, (r0, n) in enumerate(zip(wo_starts, wo_sizes)):
                late += _round_robin(row_copies(wo_hbm, wob, r0, n, s_wo + i), 4)

            start(early)
            x_copy = pltpu.make_async_copy(x_hbm, xb, sems.at[s_x])
            gw_copy = pltpu.make_async_copy(gw_hbm, gwb, sems.at[s_gw])
            x_copy.start()
            gw_copy.start()
            start_kv(0, 0, steps)

            x_copy.wait()
            gw_copy.wait()
            wait_all(wqb, s_wq)
            x1 = xb[0].astype(f32)
            gw1 = gwb[...].astype(f32).reshape(1, D)
            gate = jax.nn.sigmoid(jnp.sum(x1 * gw1, axis=-1, keepdims=True))
            xm = jnp.broadcast_to(x1, (_M, D)).astype(bf16)

            def attend(h):
                wq_h = wqb[:, pl.ds(pl.multiple_of(h * DH, DH), DH)]
                q = jnp.dot(xm, wq_h, preferred_element_type=f32).astype(bf16)
                s = lax.dot_general(q, kb[h], _NT, preferred_element_type=f32) * scale
                p = jnp.exp(s - jnp.max(s, axis=-1, keepdims=True))
                o = jnp.dot(p.astype(bf16), vb[h], preferred_element_type=f32)
                o_scr[h] = o / jnp.sum(p, axis=-1, keepdims=True)

            def group(g, _):
                start_kv(g, 0, lead_steps)
                wait_kv(g - 1)

                def head(j, _):
                    attend((g - 1) * _G + j)
                    start_kv(g, lead_steps + j * head_steps, head_steps)

                lax.fori_loop(0, _G, head, None)

            lax.fori_loop(1, n_groups, group, None)

            start(late[:_LEAD])
            wait_kv(n_groups - 1)

            def last_head(j, _):
                attend(H - _G + j)
                for jj in range(_G):
                    @pl.when(j == jj)
                    def _():
                        start(late[_LEAD + jj * _LATE_STEP:_LEAD + (jj + 1) * _LATE_STEP])

            lax.fori_loop(0, _G, last_head, None)

            o_last = o_scr[H - 1][0:1].astype(bf16).astype(f32) * gate
            ot_scr[...] = jnp.broadcast_to(o_last, (DH, DH)).T

            pos = _LEAD + _G * _LATE_STEP
            start(late[pos:pos + 32])
            wait_all(wgb, s_wg)
            gg = lax.dot_general(xm, wgb[...], _NT, preferred_element_type=f32)
            wait_all(wub, s_wu)
            uu = lax.dot_general(xm, wub[...], _NT, preferred_element_type=f32)
            hidden = (gg * jax.nn.sigmoid(gg) * uu).astype(bf16)
            start(late[pos + 32:])
            wait_all(wdb, s_wd)
            ffn = jnp.dot(hidden, wdb[...], preferred_element_type=f32)

            def project(h, acc):
                wo_h = wob[pl.ds(pl.multiple_of(h * DH, DH), DH), :]
                return acc + jnp.dot(o_scr[h].astype(bf16), wo_h, preferred_element_type=f32)

            acc = jnp.zeros((_M, D), f32)
            for i, n in enumerate(_WO_MXU):
                wait_all(wob.at[pl.ds(wo_starts[i], wo_sizes[i])], s_wo + i)
                h0 = wo_starts[i] // DH
                if n > 4:
                    acc = lax.fori_loop(h0, h0 + n, project, acc, unroll=4)
                else:
                    for h in range(h0, h0 + n):
                        acc = project(h, acc)

            row = lax.broadcasted_iota(jnp.int32, (_M, D), 0)
            part = jnp.where(row == 0, gate * acc + (1.0 - gate) * ffn, 0.0)
            for i in range(len(_WO_MXU), len(wo_sizes)):
                wait_all(wob.at[pl.ds(wo_starts[i], wo_sizes[i])], s_wo + i)
                for r in range(wo_starts[i], wo_starts[i] + wo_sizes[i], 2 * _M):
                    coef = ot_scr[pl.ds(r - (H - 1) * DH, 2 * _M), :]
                    prod = wob[pl.ds(r, 2 * _M), :].astype(f32) * jnp.concatenate(
                        [coef] * (D // DH), axis=1)
                    part = part + (prod[:_M] + prod[_M:])
            out_ref[0] = jnp.sum(part, axis=0, keepdims=True).astype(out_ref.dtype)

        pl.run_scoped(body, pltpu.SemaphoreType.DMA((s_wo + len(wo_sizes),)))

    hbm = pl.BlockSpec(memory_space=pltpu.HBM)
    return pl.pallas_call(
        kernel,
        out_shape=jax.ShapeDtypeStruct(A_x.shape, A_x.dtype),
        in_specs=[hbm] * 9,
        out_specs=pl.BlockSpec(memory_space=pltpu.VMEM),
        scratch_shapes=[
            pltpu.VMEM(A_x.shape, bf16), pltpu.VMEM(gate_w.shape, bf16),
            pltpu.VMEM((H, W, DH), bf16), pltpu.VMEM((H, W, DH), bf16),
            pltpu.VMEM(A_wq.shape, bf16), pltpu.VMEM(A_wo.shape, bf16),
            pltpu.VMEM((F, D), bf16), pltpu.VMEM((F, D), bf16), pltpu.VMEM((F, D), bf16),
            pltpu.VMEM((H, _M, DH), f32), pltpu.VMEM((DH, DH), f32),
        ],
        compiler_params=pltpu.CompilerParams(vmem_limit_bytes=100 * 1024 * 1024),
    )(A_x, A_k_cache, A_v_cache, A_wq, A_wo, B_w_gate.T, B_w_up.T, B_w_down, gate_w)
```

```python
import jax
import jax.numpy as jnp
from jax import lax
import jax.experimental.pallas as pl
import jax.experimental.pallas.tpu as pltpu

_NT = (((1,), (1,)), ((), ()))
_M = 8
_GROUP = 8
_KV_ROWS = 64
_W_ROWS = 32
_WQ_COLS = 2048
_LEAD_STEPS = 16
_LATE_BURST = 38
_QUEUE1_LAG = 25
_WO_MXU = (16, 8, 4, 2, 1)
_WO_VPU = (96, 32)


def _round_robin(items, ways):
    run = -(-len(items) // ways)
    return [items[j] for i in range(run) for j in range(i, len(items), run)]


def _land_in_order(items):
    by_landing = sorted(range(len(items)), key=lambda j: j + 2 * _QUEUE1_LAG * (j % 2))
    slots = [None] * len(items)
    for item, j in zip(items, by_landing):
        slots[j] = (item, j % 2)
    return slots


@jax.jit
def pallas_gated_mix__sliding_block_cached__swiglu_ffn__decode_kernel(
    A_x: jax.Array,
    A_k_cache: jax.Array,
    A_v_cache: jax.Array,
    A_wq: jax.Array,
    A_wo: jax.Array,
    B_x: jax.Array,
    B_w_gate: jax.Array,
    B_w_up: jax.Array,
    B_w_down: jax.Array,
    gate_w: jax.Array,
):
    del B_x
    f32, bf16 = jnp.float32, jnp.bfloat16
    _, _, D = A_x.shape
    _, H, SK, DH = A_k_cache.shape
    F = B_w_down.shape[0]
    W = min(4096, max(256, SK // 4))
    scale = DH ** -0.5

    n_groups = H // _GROUP
    pairs = _GROUP // 2
    burst_steps = (W // _KV_ROWS - _LEAD_STEPS) // pairs
    assert n_groups * _GROUP == H and (_LEAD_STEPS + pairs * burst_steps) * _KV_ROWS == W
    assert sum(_WO_MXU) == H - 1 and sum(_WO_VPU) == DH and F % _W_ROWS == 0
    mxu_starts = [sum(_WO_MXU[:i]) for i in range(len(_WO_MXU))]
    vpu_starts = [sum(_WO_VPU[:i]) for i in range(len(_WO_VPU))]
    s_wq, s_x, s_gw, s_wg, s_wu, s_wd, s_mxu = range(2 * n_groups, 2 * n_groups + 7)
    s_vpu = s_mxu + len(_WO_MXU)

    def wo_head(n, j):
        return (H // n) // 2 - 1 + j * (H // n)

    assert sorted(wo_head(n, j) for n in _WO_MXU for j in range(n)) == list(range(H - 1))

    def kernel(x_hbm, k_hbm, v_hbm, wq_hbm, wo_hbm, wg_hbm, wu_hbm, wd_hbm, gw_hbm, out_ref,
               xb, gwb, kb, vb, wqb, wob, wgb, wub, wdb, q_scr, o_scr, ot_scr):
        def body(sems):
            def start(copies):
                for (src, dst, s), queue in copies:
                    pltpu.make_async_copy(src, dst, sems.at[s]).start(priority=queue)

            def wait_all(buf, s):
                pltpu.make_async_copy(buf, buf, sems.at[s]).wait()

            def row_copies(src, dst, first, n, s):
                return [(src.at[pl.ds(r, _W_ROWS)], dst.at[pl.ds(r, _W_ROWS)], s)
                        for r in range(first, first + n, _W_ROWS)]

            def start_kv(g, first, n):
                def step(i, _):
                    r = pl.multiple_of(i * _KV_ROWS, _KV_ROWS)
                    for pair in range(pairs):
                        heads = pl.ds(g * _GROUP + 2 * pair, 2)
                        for j, (src, dst) in enumerate(((k_hbm, kb), (v_hbm, vb))):
                            pltpu.make_async_copy(
                                src.at[0, heads, pl.ds(SK - W + r, _KV_ROWS), :],
                                dst.at[heads, pl.ds(r, _KV_ROWS), :],
                                sems.at[2 * g + j],
                            ).start(priority=j)

                lax.fori_loop(first, first + n, step, None)

            def wait_kv(g):
                wait_all(kb.at[pl.ds(g * _GROUP, _GROUP)], 2 * g)
                wait_all(vb.at[pl.ds(g * _GROUP, _GROUP)], 2 * g + 1)

            early = _round_robin(
                [(wq_hbm.at[t, :, pl.ds(c, _WQ_COLS)], wqb.at[t, :, pl.ds(c, _WQ_COLS)], s_wq)
                 for t in range(D // 8) for c in range(0, H * DH, _WQ_COLS)], 8)
            wo_slices = [
                [copy for j in range(n) for copy in row_copies(
                    wo_hbm.at[wo_head(n, j)], wob.at[mxu_starts[i] + j], 0, DH, s_mxu + i)]
                for i, n in enumerate(_WO_MXU)]
            late = _round_robin(
                row_copies(wg_hbm, wgb, 0, F, s_wg) + row_copies(wu_hbm, wub, 0, F, s_wu), 6)
            late += _round_robin(row_copies(wd_hbm, wdb, 0, F, s_wd) + wo_slices[0], 7)
            for n, copies in zip(_WO_MXU[1:], wo_slices[1:]):
                late += _round_robin(copies, n)
            for i, n in enumerate(_WO_VPU):
                late += row_copies(wo_hbm.at[H - 1], wob.at[H - 1], vpu_starts[i], n, s_vpu + i)
            late = _land_in_order(late)

            start([(copy, 1 if j <= _QUEUE1_LAG else j % 2) for j, copy in enumerate(early)])
            x_copy = pltpu.make_async_copy(x_hbm, xb, sems.at[s_x])
            gw_copy = pltpu.make_async_copy(gw_hbm, gwb, sems.at[s_gw])
            x_copy.start(priority=0)
            gw_copy.start(priority=1)
            start_kv(0, 0, _LEAD_STEPS)

            x_copy.wait()
            gw_copy.wait()
            wait_all(wqb, s_wq)
            x1 = xb[0].astype(f32)
            gw1 = gwb[...].astype(f32).reshape(1, D)
            gate = jax.nn.sigmoid(jnp.sum(x1 * gw1, axis=-1, keepdims=True))
            xm = jnp.broadcast_to(x1, (_M, D)).astype(bf16)

            def project_q(j, _):
                for u in range(H // pairs):
                    h = j * (H // pairs) + u
                    wq_h = wqb[:, :, pl.ds(pl.multiple_of(h * DH, DH), DH)].reshape(D, DH)
                    q_scr[h] = jnp.dot(xm, wq_h, preferred_element_type=f32)
                start_kv(0, _LEAD_STEPS + j * burst_steps, burst_steps)

            lax.fori_loop(0, pairs, project_q, None)

            def attend_pair(h0):
                heads = (h0, h0 + 1)
                scores = [lax.dot_general(q_scr[h].astype(bf16), kb[h], _NT,
                                          preferred_element_type=f32) * scale for h in heads]
                for h, s in zip(heads, scores):
                    p = jnp.exp(s - jnp.max(s, axis=-1, keepdims=True))
                    o = jnp.dot(p.astype(bf16), vb[h], preferred_element_type=f32)
                    o_scr[h] = o / jnp.sum(p, axis=-1, keepdims=True)

            def group(g, _):
                start_kv(g, 0, _LEAD_STEPS)
                wait_kv(g - 1)

                def pair(j, _):
                    attend_pair((g - 1) * _GROUP + 2 * j)
                    start_kv(g, _LEAD_STEPS + j * burst_steps, burst_steps)

                lax.fori_loop(0, pairs, pair, None)

            lax.fori_loop(1, n_groups, group, None)

            late_lead = len(late) - pairs * _LATE_BURST
            assert late_lead >= 0
            start(late[:late_lead])
            wait_kv(n_groups - 1)

            def last_pair(j, _):
                attend_pair(H - _GROUP + 2 * j)
                for jj in range(pairs):
                    @pl.when(j == jj)
                    def _():
                        first = late_lead + jj * _LATE_BURST
                        start(late[first:first + _LATE_BURST])

            lax.fori_loop(0, pairs, last_pair, None)

            o_last = o_scr[H - 1][0:1].astype(bf16).astype(f32) * gate
            ot_scr[...] = jnp.broadcast_to(o_last, (DH, DH)).T

            wait_all(wgb, s_wg)
            gg = lax.dot_general(xm, wgb[...], _NT, preferred_element_type=f32)
            wait_all(wub, s_wu)
            uu = lax.dot_general(xm, wub[...], _NT, preferred_element_type=f32)
            hidden = (gg * jax.nn.sigmoid(gg) * uu).astype(bf16)
            wait_all(wdb, s_wd)
            ffn = jnp.dot(hidden, wdb[...], preferred_element_type=f32)

            attn = jnp.zeros((_M, D), f32)
            for i, n in enumerate(_WO_MXU):
                def project_o(j, acc):
                    return acc + jnp.dot(o_scr[wo_head(n, j)].astype(bf16), wob[mxu_starts[i] + j],
                                         preferred_element_type=f32)

                wait_all(wob.at[pl.ds(mxu_starts[i], n)], s_mxu + i)
                if n > 4:
                    attn = lax.fori_loop(0, n, project_o, attn, unroll=4)
                else:
                    for j in range(n):
                        attn = project_o(j, attn)

            row = lax.broadcasted_iota(jnp.int32, (_M, D), 0)
            part = jnp.where(row == 0, gate * attn + (1.0 - gate) * ffn, 0.0)
            for i, n in enumerate(_WO_VPU):
                wait_all(wob.at[H - 1, pl.ds(vpu_starts[i], n)], s_vpu + i)
                for r in range(vpu_starts[i], vpu_starts[i] + n, 2 * _M):
                    coef = jnp.concatenate([ot_scr[pl.ds(r, 2 * _M), :]] * (D // DH), axis=1)
                    prod = wob[H - 1, pl.ds(r, 2 * _M), :].astype(f32) * coef
                    part = part + (prod[:_M] + prod[_M:])
            out_ref[0] = jnp.sum(part, axis=0, keepdims=True).astype(out_ref.dtype)

        pl.run_scoped(body, pltpu.SemaphoreType.DMA((s_vpu + len(_WO_VPU),)))

    hbm = pl.BlockSpec(memory_space=pltpu.HBM)
    wq_shape, wo_shape = (D // 8, 8, H * DH), (H, DH, D)
    return pl.pallas_call(
        kernel,
        out_shape=jax.ShapeDtypeStruct(A_x.shape, A_x.dtype),
        in_specs=[hbm] * 9,
        out_specs=pl.BlockSpec(memory_space=pltpu.VMEM),
        scratch_shapes=[
            pltpu.VMEM(A_x.shape, bf16), pltpu.VMEM(gate_w.shape, bf16),
            pltpu.VMEM((H, W, DH), bf16), pltpu.VMEM((H, W, DH), bf16),
            pltpu.VMEM(wq_shape, bf16), pltpu.VMEM(wo_shape, bf16),
            pltpu.VMEM((F, D), bf16), pltpu.VMEM((F, D), bf16), pltpu.VMEM((F, D), bf16),
            pltpu.VMEM((H, _M, DH), f32), pltpu.VMEM((H, _M, DH), f32), pltpu.VMEM((DH, DH), f32),
        ],
        compiler_params=pltpu.CompilerParams(vmem_limit_bytes=100 * 1024 * 1024),
    )(A_x, A_k_cache, A_v_cache, A_wq.reshape(wq_shape), A_wo.reshape(wo_shape),
      B_w_gate.T, B_w_up.T, B_w_down, gate_w)
```
